```python
import os as _os
_os.environ.setdefault("JAX_PLATFORMS", "cpu")
import jax
import jax.numpy as jnp

def _softmax(x, axis=-1):
    return jax.nn.softmax(x, axis=axis)
def _gelu(x):
    return jax.nn.gelu(x, approximate=True)
def _silu(x):
    return jax.nn.silu(x)
def _sigmoid(x):
    return jax.nn.sigmoid(x)
def _layernorm(x, axis=-1, eps=1e-5):
    m = jnp.mean(x, axis=axis, keepdims=True)
    v = jnp.var(x, axis=axis, keepdims=True)
    return (x - m) / jnp.sqrt(v + eps)
def _scatter_add(tgt, idx, src, axis=0):
    return tgt.at[idx].add(src)
def _segment_sum(src, seg, n):
    return jax.ops.segment_sum(src, seg, n)
class _Rng:
    def __init__(self, key):
        self._k = key
    def _next(self):
        self._k, sub = jax.random.split(self._k)
        return sub
    def normal(self, shape):
        return jax.random.normal(self._next(), shape, dtype=jnp.bfloat16)
    def randint(self, lo, hi, shape):
        return jax.random.randint(self._next(), shape, lo, hi, dtype=jnp.int32)
    def uniform(self, shape, lo=0.0, hi=1.0):
        return jax.random.uniform(self._next(), shape, jnp.bfloat16, lo, hi)
    def permutation(self, n):
        return jax.random.permutation(self._next(), n)


kernel_name = 'concat_heads__gqa_block_cached__mha_block_cached__near_ridge'

def setup_inputs():
    _rng = _Rng(jax.random.key(int.from_bytes(__import__("os").urandom(4), "little")))
    _w = (lambda a: (lambda t: t.astype(jnp.bfloat16) if jnp.issubdtype(t.dtype, jnp.floating) else t)(jnp.asarray(a)))
    def _A_setup():
        B, Sq, D = 8, 112, 448
        Hq, Hkv, Sk, Dh = 16, 8, 512, 256
        assert Hq % Hkv == 0, (Hq, Hkv)
        return {
            "x": _w((lambda *s: _rng.normal(s) * 0.8)(B, Sq, D)),
            "k_cache": _w((lambda *s: _rng.normal(s) * 0.8)(B, Hkv, Sk, Dh)),
            "v_cache": _w((lambda *s: _rng.normal(s) * 0.05)(B, Hkv, Sk, Dh)),
            "wq": _w((lambda *s: _rng.normal(s) * 0.8)(D, Hq * Dh) * (D ** -0.5)),
            "wo": _w((lambda *s: _rng.normal(s) * 0.05)(Hq * Dh, D) * ((Hq * Dh) ** -0.5)),
        }
    _A_in = _A_setup()

    def _B_setup():
        B, Sq, D = 8, 112, 448
        H, Sk, Dh = 16, 512, 256
        return {
            "x": _w((lambda *s: _rng.normal(s) * 0.8)(B, Sq, D)),
            "k_cache": _w((lambda *s: _rng.normal(s) * 0.8)(B, H, Sk, Dh)),
            "v_cache": _w((lambda *s: _rng.normal(s) * 0.05)(B, H, Sk, Dh)),
            "wq": _w((lambda *s: _rng.normal(s) * 0.8)(D, H * Dh) * (D ** -0.5)),
            "wo": _w((lambda *s: _rng.normal(s) * 0.05)(H * Dh, D) * ((H * Dh) ** -0.5)),
        }
    _B_in = _B_setup()

    return {
        "A_x": _A_in["x"],
        "A_k_cache": _A_in["k_cache"],
        "A_v_cache": _A_in["v_cache"],
        "A_wq": _A_in["wq"],
        "A_wo": _A_in["wo"],
        "B_x": _B_in["x"],
        "B_k_cache": _B_in["k_cache"],
        "B_v_cache": _B_in["v_cache"],
        "B_wq": _B_in["wq"],
        "B_wo": _B_in["wo"],
    }

def reference(A_x, A_k_cache, A_v_cache, A_wq, A_wo, B_x, B_k_cache, B_v_cache, B_wq, B_wo):
    def _A_ref(x, k_cache, v_cache, wq, wo):
        B, Sq, D = x.shape
        Hq, Dh = 16, 256
        Hkv = k_cache.shape[1]
        rep = Hq // Hkv
        q = (lambda x, *d: x.transpose(*d))((x @ wq).reshape(B, Sq, Hq, Dh), 0, 2, 1, 3)
        k = jnp.repeat(k_cache, rep, axis=1)
        v = jnp.repeat(v_cache, rep, axis=1)
        scores = jnp.einsum("bhqd,bhkd->bhqk", q, k) * (Dh ** -0.5)
        p = _softmax(scores, axis=-1)
        o = jnp.einsum("bhqk,bhkd->bhqd", p, v)
        return (lambda x, *d: x.transpose(*d))(o, 0, 2, 1, 3).reshape(B, Sq, Hq * Dh) @ wo

    def _B_ref(x, k_cache, v_cache, wq, wo):
        B, Sq, D = x.shape
        H, Dh = 16, 256
        q = (lambda x, *d: x.transpose(*d))((x @ wq).reshape(B, Sq, H, Dh), 0, 2, 1, 3)
        scores = jnp.einsum("bhqd,bhkd->bhqk", q, k_cache) * (Dh ** -0.5)
        p = _softmax(scores, axis=-1)
        o = jnp.einsum("bhqk,bhkd->bhqd", p, v_cache)
        return (lambda x, *d: x.transpose(*d))(o, 0, 2, 1, 3).reshape(B, Sq, H * Dh) @ wo

    a = _A_ref(A_x, A_k_cache, A_v_cache, A_wq, A_wo)
    b = _B_ref(B_x, B_k_cache, B_v_cache, B_wq, B_wo)
    return jnp.concatenate([a, b], axis=-1)
```

```python
import jax
import jax.numpy as jnp
import jax.experimental.pallas as pl
import jax.experimental.pallas.tpu as pltpu

NT = (((1,), (1,)), ((), ()))
F32, BF16 = jnp.float32, jnp.bfloat16
LAG = 4
NCH = (1, 1, 2, 4)
EARLY = 8
NODMA = False
SCOPES = False
WSPLIT = (0, 5, 6, 7)
SA = "Q0 W0 K0 V0 k0 k1 k2 s0 q0 s1 v0 v1 k3 k4 q1 o0 s2 s3 q2 v2 k5 v3 o1 s4 q3 v4 s5 k6 o2 q4 v5 k7 o3 s6 q5 v6 s7 o4 v7 q7 o5 o6 q6"
SB = None
SN = "W0 K0 V0 k0 k1 s0 k2 s1 v0 k3 s2 v1 K1 V1 k4 v2 s3 k5 o0 v3 s4 k6 o1 v4 s5 k7 o2 v5 s6 o3 v6 s7 o4 v7 o5 o6"
SF = "W0 K0 V0 k0 k1 s0 s1 v0 v1 K1 V1 k2 k3 o0 s2 s3 v2 T0 v3 K2 V2 k4 k5 o1 s4 o2 s5 v4 T1 v5 T2 K3 k6 k7 o3 s6 o4 s7 T3 T4 V3 X0 v6 v7 o5 T5 X1 o6 T6 X2"
FLAGS = {}
NOSEM = True
ONLY = 'abnf'


@jax.jit
def pallas_concat_heads__gqa_block_cached__mha_block_cached__near_ridge_kernel(
    A_x, A_k_cache, A_v_cache, A_wq, A_wo, B_x, B_k_cache, B_v_cache, B_wq, B_wo):
    B, Sq, D = A_x.shape
    _, G, Sk, Dh = A_k_cache.shape
    M = B * Sq
    W = 2 * Dh
    TT = 128

    def scope(name, fn):
        if SCOPES:
            with jax.named_scope(name):
                return fn()
        return fn()

    def kern(xa, ka, va, wqa, woa, xb, kb, vb, wqb, wob, out,
             x, wq, wo, kA, vA, kB, vB, q, o, acc, ostage, xsem, wsem, asem, bsem, osem):
        def x_copy(i):
            return pltpu.make_async_copy((xa, xb)[i], x.at[i], xsem.at[i])

        def w_copy(br, which, g):
            src, dst = ((wqa, woa), (wqb, wob))[br][which], (wq, wo)[which]
            start = g * W if isinstance(g, int) else pl.multiple_of(g * W, W)
            return pltpu.make_async_copy(src.at[:, pl.ds(start, W)], dst.at[br * G + g], wsem.at[which, br * G + g])

        def kv_copy(kind, which, g, c):
            n = B // NCH[kind]
            bs = pl.ds(c * n, n)
            if kind == 0:
                return pltpu.make_async_copy((ka, va)[which].at[bs, g], (kA, vA)[which].at[g, bs], asem.at[which, g, c])
            return pltpu.make_async_copy((kb, vb)[which].at[bs, pl.ds(2 * g, 2)], (kB, vB)[which].at[g, bs], bsem.at[which, g, c])

        def loop(lo, hi, fn):
            jax.lax.fori_loop(lo, hi, lambda i, c: (fn(i), c)[1], 0)

        def issue(kind, g):
            br = min(kind, 1)
            if kind == 0:
                pl.when(g + LAG < G)(lambda: w_copy(0, 0, g + LAG).start())
                pl.when(g + LAG == G)(lambda: x_copy(1).start())
                pl.when(g + LAG >= G)(lambda: w_copy(1, 0, g + LAG - G).start())
            elif kind == 1:
                w_copy(1, 0, g + LAG).start()
            w_copy(br, 1, g).start()
            def chunk(c):
                kv_copy(kind, 0, g, c).start()
                kv_copy(kind, 1, g, c).start()
            loop(0, NCH[kind], chunk)

        def qproj(n, b):
            r0 = b * Sq if isinstance(b, int) else pl.multiple_of(b * Sq, 16)
            r = jnp.dot(x[n // G, pl.ds(r0, Sq), :], wq[n], preferred_element_type=F32)
            r = (r * (Dh ** -0.5)).astype(BF16)
            q[n % LAG, b, 0:Sq, :] = r[:, 0:Dh]
            q[n % LAG, b, Sq:2 * Sq, :] = r[:, Dh:W]

        def wq_wait(n):
            pltpu.make_async_copy(wq.at[n], wq.at[n], wsem.at[0, n]).wait()

        def out_copy(i):
            rows = pl.ds(WSPLIT[i] * TT, (WSPLIT[i + 1] - WSPLIT[i]) * TT)
            return pltpu.make_async_copy(ostage.at[rows], out.at[rows], osem.at[i])

        def pair(kind, g, sched):
            br = min(kind, 1)
            n = br * G + g
            st = {}
            for tok in sched.split():
                op, b = tok[0], int(tok[1])
                ts = [int(tok[2])] if len(tok) > 2 else [0, 1]
                rows = slice(b * Sq, (b + 1) * Sq)
                cols = slice(b * TT, (b + 1) * TT)
                if op in "KVWQ":
                    if NODMA:
                        continue
                    if op == "Q":
                        wq_wait(n + LAG)
                        if kind == 0:
                            pl.when(g + LAG == G)(lambda: x_copy(1).wait())
                    else:
                        (w_copy(br, 1, g) if op == "W" else kv_copy(kind, "KV".index(op), g, b)).wait()
                elif op == "q":
                    qproj(n + LAG, b)
                elif op == "k":
                    if br == 0:
                        st[b, 0] = jax.lax.dot_general(q[n % LAG, b], kA[g, b], NT, preferred_element_type=F32)
                    else:
                        for t in ts:
                            st[b, t] = jax.lax.dot_general(q[n % LAG, b, t * Sq:(t + 1) * Sq, :], kB[g, b, t], NT,
                                                           preferred_element_type=F32)
                elif op == "s":
                    for t in ([0] if br == 0 else ts):
                        s = st[b, t]
                        p = jnp.exp(s - jnp.max(s, axis=-1, keepdims=True))
                        st[b, t] = (p.astype(BF16), jnp.sum(p, axis=-1, keepdims=True))
                elif op == "v":
                    if br == 0:
                        p, l = st.pop((b, 0))
                        r = (jnp.dot(p, vA[g, b], preferred_element_type=F32) * (1.0 / l)).astype(BF16)
                        o[rows, 0:Dh] = r[0:Sq]
                        o[rows, Dh:W] = r[Sq:2 * Sq]
                    else:
                        for t in ts:
                            p, l = st.pop((b, t))
                            r = jnp.dot(p, vB[g, b, t], preferred_element_type=F32) * (1.0 / l)
                            o[rows, t * Dh:(t + 1) * Dh] = r.astype(BF16)
                elif op == "o":
                    acc[br * D:(br + 1) * D, cols] += jax.lax.dot_general(
                        wo[n], o[cols, :], NT, preferred_element_type=F32)
                elif op == "T":
                    ostage[cols, :] = acc[:, cols].astype(BF16).T
                elif op == "X":
                    out_copy(b).start()

        def issue_b(lo, hi):
            loop(lo, max(lo, min(hi, G - LAG)), lambda g: issue(1, g))
            loop(max(lo, G - LAG), max(lo, G - LAG, min(hi, G - 1)), lambda g: issue(2, g))
            if lo < G and hi == G:
                issue(3, G - 1)

        def start_dmas():
            x_copy(0).start()
            loop(0, LAG, lambda g: w_copy(0, 0, g).start())
            loop(0, G, lambda g: issue(0, g))
            issue_b(0, EARLY)

        def prologue():
            acc[...] = jnp.zeros_like(acc)
            if not NODMA:
                x_copy(0).wait()

        def qpair(n):
            if not NODMA:
                wq_wait(n)
            for b in range(B):
                qproj(n, b)

        if not NODMA:
            scope("z_i", start_dmas)
        scope("z_w", prologue)
        if len(ONLY) > 1: loop(0, LAG, lambda n: scope("z_q", lambda: qpair(n)))
        if "a" in ONLY: loop(0, G, lambda g: scope("z_a", lambda: pair(0, g, SA)))
        if not NODMA:
            issue_b(EARLY, G)
        if "b" in ONLY: loop(0, G - LAG, lambda g: scope("z_b", lambda: pair(1, g, SB or SA)))
        if "n" in ONLY: loop(G - LAG, G - 1, lambda g: scope("z_n", lambda: pair(2, g, SN)))
        if "f" in ONLY: scope("z_f", lambda: pair(3, G - 1, SF))
        scope("z_e", lambda: [out_copy(i).wait() for i in range(len(WSPLIT) - 1)])

    hbm = pl.BlockSpec(memory_space=pltpu.MemorySpace.HBM)
    res = pl.pallas_call(
        kern, in_specs=[hbm] * 10, out_specs=hbm,
        out_shape=jax.ShapeDtypeStruct((M, 2 * D), BF16),
        scratch_shapes=[
            pltpu.VMEM((2, M, D), BF16), pltpu.VMEM((2 * G, D, W), BF16), pltpu.VMEM((2 * G, D, W), BF16),
            pltpu.VMEM((G, B, Sk, Dh), BF16), pltpu.VMEM((G, B, Sk, Dh), BF16),
            pltpu.VMEM((G, B, 2, Sk, Dh), BF16), pltpu.VMEM((G, B, 2, Sk, Dh), BF16),
            pltpu.VMEM((LAG, B, 2 * Sq, Dh), BF16), pltpu.VMEM((M, W), BF16), pltpu.VMEM((2 * D, M), F32),
            pltpu.VMEM((M, 2 * D), BF16),
            pltpu.SemaphoreType.DMA((2,)), pltpu.SemaphoreType.DMA((2, 2 * G)), pltpu.SemaphoreType.DMA((2, G, NCH[0])),
            pltpu.SemaphoreType.DMA((2, G, max(NCH))), pltpu.SemaphoreType.DMA((len(WSPLIT) - 1,))],
        compiler_params=pltpu.CompilerParams(vmem_limit_bytes=127 * 2**20, flags=FLAGS or None, disable_bounds_checks=True, disable_semaphore_checks=NOSEM),
    )(A_x.reshape(M, D), A_k_cache, A_v_cache, A_wq, A_wo.T, B_x.reshape(M, D), B_k_cache, B_v_cache, B_wq, B_wo.T)
    return res.reshape(B, Sq, 2 * D)
```

```python
import jax
import jax.numpy as jnp
import jax.experimental.pallas as pl
import jax.experimental.pallas.tpu as pltpu

NT = (((1,), (1,)), ((), ()))
F32, BF16 = jnp.float32, jnp.bfloat16
LOG2E = 1.4426950408889634
TT = 128
LAG = 4
LOOK = 3
WLOOK = 2
WROWS = 32
XB = 3
VLAST = (0, 4, 6, 8)
OSPLIT = (0, 5, 6, 7)

SA = "W0 K0 k0 k1 q0 s0 s1 v1 k2 k3 q2 s2 s3 v0 q1 o0 k4 v2 s4 k5 s5 o1 v3 v4 k6 q3 q4 o3 o2 k7 q5 v5 s6 v6 o4 s7 v7 q6 q7 o6 o5"
SB = "W0 K0 k0 A0 k1 k2 q0 s0 v0 k3 s1 v1 k4 s2 q1 q2 s3 v2 o0 v3 k5 s4 o1 k6 v4 q4 q3 A1 o2 s6 o3 s5 v5 k7 q5 v6 o4 s7 v7 q6 o6 o5 A2 q7"
SM = "W0 K0 k0 A0 k1 k2 s0 s1 v0 k3 v1 s3 s2 k4 o0 s4 v2 k5 v3 k6 o1 A1 v4 k7 s5 o2 v5 s7 s6 o3 v6 o4 v7 A2 o5 o6"
SN = "W0 K0 k0 A0 k1 k2 s0 v0 k3 s1 s3 s2 v1 v2 o0 v3 o1 K1 k4 A1 k5 o2 k6 k7 s5 s4 v4 s6 v5 s7 o3 o4 A2 v6 v7 o5 o6"
SF = "W0 K0 k0 k2 k1 s2 s0 v0 k3 s3 s1 v1 v2 z0 v3 K1 k4 s4 z2 k5 z1 k6 k7 s6 X0 V0 s5 v4 v5 z3 z4 s7 X1 V1 v6 v7 z5 X2 z6 X3"


@jax.jit
def pallas_concat_heads__gqa_block_cached__mha_block_cached__near_ridge_kernel(
    A_x: jax.Array,
    A_k_cache: jax.Array,
    A_v_cache: jax.Array,
    A_wq: jax.Array,
    A_wo: jax.Array,
    B_x: jax.Array,
    B_k_cache: jax.Array,
    B_v_cache: jax.Array,
    B_wq: jax.Array,
    B_wo: jax.Array,
):
    B, Sq, D = A_x.shape
    _, G, Sk, Dh = A_k_cache.shape
    assert (B, G) == (8, 8) and B * Sq == 7 * TT and B_k_cache.shape == (B, 2 * G, Sk, Dh)
    M, W, HB, N = B * Sq, 2 * Dh, B // 2, 2 * G
    F0 = D // TT * TT
    KP = 4

    def aligned(i, n):
        return i if isinstance(i, int) else pl.multiple_of(i, n)

    def kernel(xa, ka, va, wqa, woa, xb, kb, vb, wqb, wob, out,
               x, w, kv, q, o, acc, ostage, xsem, wsem, kvsem, osem):

        def loop(lo, hi, fn):
            jax.lax.fori_loop(lo, hi, lambda i, c: (fn(i), c)[1], 0)

        def wait_for(ref, sem):
            pltpu.make_async_copy(ref, ref, sem).wait()

        def x_copy(i):
            if i == 2:
                return pltpu.make_async_copy(xb, x.at[1], xsem.at[2])
            rows = (pl.ds(0, XB * Sq), pl.ds(XB * Sq, M - XB * Sq))[i]
            return pltpu.make_async_copy(xa.at[rows], x.at[0, rows], xsem.at[i])

        def wq0_copy(t):
            cols = pl.ds(t * Dh, Dh)
            return pltpu.make_async_copy(wqa.at[:, cols], w.at[0, 0, :, cols], xsem.at[3 + t])

        def w_copy(br, which, m, rows):
            src = ((wqa, woa), (wqb, wob))[br][which]
            slot = (m + which * LAG) % N
            return pltpu.make_async_copy(src.at[rows, pl.ds(aligned((m - br * G) * W, W), W)],
                                         w.at[slot, which, rows], wsem.at[slot])

        def w_piece(which, m, lo, hi, u):
            for br in range(2):
                if u >= D // WROWS or hi <= br * G or lo >= (br + 1) * G:
                    continue
                start = lambda: w_copy(br, which, m, pl.ds(u * WROWS, WROWS)).start()
                if lo >= br * G and hi <= (br + 1) * G:
                    start()
                else:
                    pl.when(jnp.logical_and(m >= br * G, m < (br + 1) * G))(start)

        def unit_sem(u):
            return kvsem.at[jnp.where(u < N - 4, u // 2 * 2, u)]

        def kb_piece(u, c):
            b, t, rows = c // (2 * KP), c // KP % 2, pl.ds(c % KP * (Sk // KP), Sk // KP)
            pltpu.make_async_copy(kb.at[u % 2 * HB + b, u // 2 * 2 + t, rows], kv.at[u, 0, b, t, rows],
                                  unit_sem(u)).start()

        def kb_unit(u):
            pltpu.make_async_copy(kb.at[pl.ds(u % 2 * HB, HB), pl.ds(u // 2 * 2, 2)], kv.at[u, 0],
                                  kvsem.at[u]).start(priority=1)

        def bulk(m, part, lo, hi):
            def a_copy():
                pltpu.make_async_copy((ka, va)[part].at[:, :, m], kv.at[N + m, part],
                                      kvsem.at[N + m]).start(priority=1)

            def b_copy():
                u = 2 * (m - G) + part
                pltpu.make_async_copy(vb.at[pl.ds(part * HB, HB), pl.ds(2 * (m - G), 2)], kv.at[u, 1],
                                      unit_sem(u)).start(priority=1)

            if hi <= G:
                a_copy()
            elif lo >= G:
                b_copy()
            else:
                if part == 0:
                    pl.when(m + LAG == G)(lambda: x_copy(2).start(priority=1))
                pl.when(m < G)(a_copy)
                pl.when(m >= G)(b_copy)

        def v_last(c):
            b0, nb = VLAST[c], VLAST[c + 1] - VLAST[c]
            return pltpu.make_async_copy(vb.at[pl.ds(b0, nb), pl.ds(N - 2, 2)],
                                         kv.at[N - 2 + b0 // HB, 1, pl.ds(b0 % HB, nb)],
                                         kvsem.at[N - 2 if c == 0 else N + G + c - 1])

        def out_copy(i):
            if i == 0:
                idx = (slice(None), pl.ds(0, F0))
            else:
                idx = (pl.ds(OSPLIT[i - 1] * TT, (OSPLIT[i] - OSPLIT[i - 1]) * TT), pl.ds(F0, 2 * D - F0))
            return pltpu.make_async_copy(ostage.at[idx], out.at[idx], osem.at[i])

        def qproj(n, b, lo, hi, pieces):
            halves = []
            for t in range(2):
                for u in pieces[t * len(pieces) // 2:(t + 1) * len(pieces) // 2]:
                    w_piece(0, n + WLOOK, lo + WLOOK, hi + WLOOK, u)
                halves.append(w[n, 0, :, t * Dh:(t + 1) * Dh])
            r = jnp.dot(x[n // G, b * Sq:(b + 1) * Sq, :], jnp.concatenate(halves, axis=1),
                        preferred_element_type=F32).astype(BF16)
            q[n % LAG, b, 0:Sq, :] = r[:, 0:Dh]
            q[n % LAG, b, Sq:2 * Sq, :] = r[:, Dh:W]

        def pair(n, lo, hi, sched):
            br = lo // G
            g = n - br * G
            with_q = lo + LAG < N
            ws = n + LAG if with_q else n + LAG - N
            site = [-1 if lo < N - 2 else 0]

            def copies():
                c = site[0]
                site[0] += 1
                if c >= 0 and br == 0:
                    pl.when(n > 0)(lambda: kb_piece(n, c))
                elif c >= 0 and lo < N - 1:
                    kb_piece(n, c)
                if with_q and c in (2, 4):
                    bulk(n + LOOK, c // 2 - 1, lo + LOOK, hi + LOOK)
                if br == 0 and c == 6:
                    pl.when(n + LOOK == G)(lambda: kb_unit(0))
                if lo + LAG == N and c in (0, 2, 4, 6):
                    pl.when(n == lo)(lambda: kb_unit(N - 1) if c == 2
                                     else v_last(max(c // 2 - 1, 0)).start(priority=1))

            def cache(which, b, t):
                if br == 1:
                    copies()
                    return kv[2 * g + b // HB, which, b % HB, t]
                ref, halves = kv.at[N + g, which, b // 2, b % 2], []
                for i in range(2):
                    copies()
                    halves.append(ref[i * Sk // 2:(i + 1) * Sk // 2, :] if which == 0
                                  else ref[:, i * Dh // 2:(i + 1) * Dh // 2])
                return jnp.concatenate(halves, axis=which)

            live = {}
            heads = (0,) if br == 0 else (0, 1)
            for tok in sched.split():
                op, b = tok[0], int(tok[1])
                rows, tile = slice(b * Sq, (b + 1) * Sq), slice(b * TT, (b + 1) * TT)
                if op == "W":
                    wait_for(w.at[ws] if with_q else w.at[ws, 1], wsem.at[ws])
                    if br == 0:
                        pl.when(n + LAG == G)(lambda: x_copy(2).wait())
                elif op == "K":
                    if br == 0:
                        wait_for(kv.at[N + g], kvsem.at[N + g])
                    elif lo < N - 2:
                        wait_for(kv.at[pl.ds(2 * g, 2)], kvsem.at[2 * g])
                    elif lo == N - 1 and b == 1:
                        wait_for(kv.at[N - 1, 0], kvsem.at[N - 1])
                    else:
                        wait_for(kv.at[2 * g + b], kvsem.at[2 * g + b])
                elif op == "V":
                    v_last(b + 1).wait()
                elif op == "q":
                    qproj(n + LAG, b, lo + LAG, hi + LAG, (2 * b, 2 * b + 1))
                elif op == "k":
                    for t in heads:
                        qt = q[n % LAG, b] if br == 0 else q[n % LAG, b, t * Sq:(t + 1) * Sq, :]
                        live[b, t] = jax.lax.dot_general(qt, cache(0, b, t), NT, preferred_element_type=F32)
                elif op == "s":
                    for t in heads:
                        s = live[b, t]
                        p = jnp.exp2((s - jnp.max(s, axis=-1, keepdims=True)) * (Dh ** -0.5 * LOG2E))
                        live[b, t] = (p.astype(BF16), jnp.sum(p, axis=-1, keepdims=True))
                elif op == "v":
                    for t in heads:
                        p, denom = live.pop((b, t))
                        r = (jnp.dot(p, cache(1, b, t), preferred_element_type=F32) * (1.0 / denom)).astype(BF16)
                        if br == 0:
                            o[rows, 0:Dh] = r[0:Sq]
                            o[rows, Dh:W] = r[Sq:2 * Sq]
                        else:
                            o[rows, t * Dh:(t + 1) * Dh] = r
                elif op == "o":
                    for i in range(2):
                        w_piece(1, n + WLOOK, lo + WLOOK, hi + WLOOK, 2 * b + i)
                        r0, r1 = i * D // 2, (i + 1) * D // 2
                        acc[b, br * D + r0:br * D + r1, :] += jax.lax.dot_general(
                            w[ws, 1, r0:r1, :], o[tile, :], NT, preferred_element_type=F32)
                elif op == "A":
                    ostage[pl.ds(aligned(g * TT, TT), TT), tile] = acc[g, tile, :].astype(BF16).T
                elif op == "z":
                    for f in range(F0, 2 * D, 2 * TT):
                        r0, r1 = max(f - D, 0), f + 2 * TT - D
                        r = acc[b, D + r0:D + r1, :] + jax.lax.dot_general(
                            w[ws, 1, r0:r1, :], o[tile, :], NT, preferred_element_type=F32)
                        if f < D:
                            r = jnp.concatenate([acc[b, f:D, :], r], axis=0)
                        ostage[tile, f:f + 2 * TT] = r.astype(BF16).T
                elif op == "X":
                    out_copy(b).start()
            if lo < N - 2:
                copies()

        def first_copies(m):
            pl.when(m == 0)(lambda: wq0_copy(1).start())
            pl.when(m == 1)(lambda: x_copy(1).start())
            pl.when(m == 0)(lambda: w_copy(0, 0, 1, slice(None)).start(priority=1))
            pl.when(m < WLOOK)(lambda: w_copy(0, 1, m, slice(None)).start(priority=1))
            for part in range(2):
                bulk(m, part, 0, LOOK)

        def q_only(n):
            wait_for(w.at[n, 0], wsem.at[n])
            for b in range(B):
                qproj(n, b, 1, LAG, (2 * b, 2 * b + 1))

        x_copy(0).start()
        wq0_copy(0).start()
        loop(0, LOOK, first_copies)
        acc[...] = jnp.zeros_like(acc)
        x_copy(0).wait()
        for t in range(2):
            wq0_copy(t).wait()
            r = jnp.dot(x[0, 0:XB * Sq, :], w[0, 0, :, t * Dh:(t + 1) * Dh], preferred_element_type=F32).astype(BF16)
            for b in range(XB):
                q[0, b, t * Sq:(t + 1) * Sq, :] = r[b * Sq:(b + 1) * Sq]
        x_copy(1).wait()
        per = pl.cdiv(D // WROWS, B - XB)
        for b in range(XB, B):
            qproj(0, b, 0, 1, tuple(range((b - XB) * per, (b - XB + 1) * per)))
        loop(1, LAG, q_only)
        loop(0, G, lambda n: pair(n, 0, G, SA))
        loop(G, N - LAG, lambda n: pair(n, G, N - LAG, SB))
        loop(N - LAG, N - 2, lambda n: pair(n, N - LAG, N - 2, SM))
        pair(N - 2, N - 2, N - 1, SN)
        pair(N - 1, N - 1, N, SF)
        for i in range(len(OSPLIT)):
            out_copy(i).wait()

    hbm = pl.BlockSpec(memory_space=pltpu.MemorySpace.HBM)
    res = pl.pallas_call(
        kernel,
        in_specs=[hbm] * 10,
        out_specs=hbm,
        out_shape=jax.ShapeDtypeStruct((M, 2 * D), BF16),
        scratch_shapes=[
            pltpu.VMEM((2, M, D), BF16),
            pltpu.VMEM((N, 2, D, W), BF16),
            pltpu.VMEM((N + G, 2, HB, 2, Sk, Dh), BF16),
            pltpu.VMEM((LAG, B, 2 * Sq, Dh), BF16),
            pltpu.VMEM((M, W), BF16),
            pltpu.VMEM((M // TT, 2 * D, TT), F32),
            pltpu.VMEM((M, 2 * D), BF16),
            pltpu.SemaphoreType.DMA((5,)),
            pltpu.SemaphoreType.DMA((N,)),
            pltpu.SemaphoreType.DMA((N + G + len(VLAST) - 2,)),
            pltpu.SemaphoreType.DMA((len(OSPLIT),)),
        ],
        compiler_params=pltpu.CompilerParams(
            vmem_limit_bytes=128 * 2**20, disable_bounds_checks=True, disable_semaphore_checks=True),
    )(A_x.reshape(M, D), A_k_cache.reshape(HB, 2, G, Sk, Dh), A_v_cache.reshape(HB, 2, G, Sk, Dh), A_wq, A_wo.T,
      B_x.reshape(M, D), B_k_cache, B_v_cache, B_wq, B_wo.T)
    return res.reshape(B, Sq, 2 * D)
```
